```python
import jax
import jax.numpy as jnp

def _softmax(x, axis=-1):
    return jax.nn.softmax(x, axis=axis)
def _gelu(x):
    return jax.nn.gelu(x, approximate=True)
def _silu(x):
    return jax.nn.silu(x)
def _sigmoid(x):
    return jax.nn.sigmoid(x)
def _layernorm(x, axis=-1, eps=1e-5):
    m = jnp.mean(x, axis=axis, keepdims=True)
    v = jnp.var(x, axis=axis, keepdims=True)
    return (x - m) / jnp.sqrt(v + eps)
def _scatter_add(tgt, idx, src, axis=0):
    return tgt.at[idx].add(src)
def _segment_sum(src, seg, n):
    return jax.ops.segment_sum(src, seg, n)
class _Rng:
    def __init__(self, key):
        self._k = key
    def _next(self):
        self._k, sub = jax.random.split(self._k)
        return sub
    def normal(self, shape):
        return jax.random.normal(self._next(), shape, dtype=jnp.bfloat16)
    def randint(self, lo, hi, shape):
        return jax.random.randint(self._next(), shape, lo, hi, dtype=jnp.int32)
    def uniform(self, shape, lo=0.0, hi=1.0):
        return jax.random.uniform(self._next(), shape, jnp.bfloat16, lo, hi)
    def permutation(self, n):
        return jax.random.permutation(self._next(), n)


kernel_name = 'sequential_preLN__sliding_local_dilated__moe_arch_mod__prompt'

def setup_inputs():
    _rng = _Rng(jax.random.key(int.from_bytes(__import__("os").urandom(4), "little")))
    _w = (lambda a: (lambda t: t.astype(jnp.bfloat16) if jnp.issubdtype(t.dtype, jnp.floating) else t)(jnp.asarray(a)))
    def _A_setup():
        B, S, D = 1, 2048, 640
        return {
            "x": _w((lambda *s: _rng.normal(s) * 0.05)(B, S, D)),
            "wqkv": _w((lambda *s: _rng.normal(s) * 0.05)(D, 3 * D)),
            "wo": _w((lambda *s: _rng.normal(s) * 0.05)(D, D)),
        }
    _A_in = _A_setup()

    def _B_setup():
        B, S, D, F, C = 1, 2048, 640, 1536, 1
        return {
            "x": _w((lambda *s: _rng.normal(s) * 0.05)(B, S, D)),
            "w_r": _w((lambda *s: _rng.normal(s) * 0.05)(D)),
            "w_gate": _w((lambda *s: _rng.normal(s) * 0.05)(D, F)),
            "w_up": _w((lambda *s: _rng.normal(s) * 0.05)(D, F)),
            "w_down": _w((lambda *s: _rng.normal(s) * 0.05)(F, D)),
        }
    _B_in = _B_setup()

    return {
        "A_x": _A_in["x"],
        "A_wqkv": _A_in["wqkv"],
        "A_wo": _A_in["wo"],
        "B_x": _B_in["x"],
        "B_w_r": _B_in["w_r"],
        "B_w_gate": _B_in["w_gate"],
        "B_w_up": _B_in["w_up"],
        "B_w_down": _B_in["w_down"],
    }

def reference(A_x, A_wqkv, A_wo, B_x, B_w_r, B_w_gate, B_w_up, B_w_down):
    def _A_ref(x, wqkv, wo):
        B, S, D = x.shape
        H = 32; Dh = D // H
        W, dil = 8, 2
        qkv = (lambda x, *d: x.transpose(*d))((x @ wqkv).reshape(B, S, 3, H, Dh), 2, 0, 3, 1, 4)
        q, k, v = qkv[0], qkv[1], qkv[2]
        scale = Dh ** -0.5
        pos = jnp.arange(S)
        off = jnp.arange(W) * dil
        idx = pos[:, None] - off[None, :]
        mask = idx >= 0
        idx_c = jnp.where(mask, idx, 0).reshape(-1)
        kg = k[:, :, idx_c, :].reshape(B, H, S, W, Dh)
        vg = v[:, :, idx_c, :].reshape(B, H, S, W, Dh)
        logits = jnp.einsum("bhsd,bhswd->bhsw", q, kg) * scale
        logits = jnp.where(mask[None, None, :, :], logits, -1e9)
        attn = _softmax(logits, axis=-1)
        o = jnp.einsum("bhsw,bhswd->bhsd", attn, vg)
        return (lambda x, *d: x.transpose(*d))(o, 0, 2, 1, 3).reshape(B, S, D) @ wo

    def _B_ref(x, w_r, w_gate, w_up, w_down):
        B, S, D = x.shape
        C = 1
        r = x @ w_r
        idx = jnp.argsort(-r, axis=-1)[:, :C]
        idx_e = jnp.repeat(idx.reshape(B, C, 1), D, axis=2)
        x_sel = jnp.take_along_axis(x, idx_e, axis=1)
        g = _silu(x_sel @ w_gate)
        u = x_sel @ w_up
        y = (g * u) @ w_down
        r_sel = _sigmoid(jnp.take_along_axis(r, idx, axis=1))
        y = y * r_sel.reshape(B, C, 1)
        b_off = (jnp.arange(B) * S).reshape(B, 1)
        flat_idx = (idx + b_off).reshape(B * C)
        zero = (x * 0.0).reshape(B * S, D)
        upd = _scatter_add(zero, flat_idx, y.reshape(B * C, D), axis=0)
        return x + upd.reshape(B, S, D)

    x = A_x
    h = x + _A_ref(_layernorm(x, axis=-1), A_wqkv, A_wo)
    h2 = h + _B_ref(_layernorm(h, axis=-1), B_w_r, B_w_gate, B_w_up, B_w_down)
    return h2
```

```python
import functools, math
import jax, jax.numpy as jnp, numpy as np
from jax.experimental import pallas as pl
from jax.experimental.pallas import tpu as pltpu

S_, D_, H_, DH_, W_, F_ = 2048, 640, 32, 20, 8, 1536
HALO = 16
EPS = 1e-5
f32, bf16, u32, i32 = jnp.float32, jnp.bfloat16, jnp.uint32, jnp.int32
NT = (((1,), (1,)), ((), ()))
NN = (((1,), (0,)), ((), ()))

def interleave(*lists):
    lists = [l for l in lists if l]
    tot = [sum(w for w, _ in l) for l in lists]
    pos = [0] * len(lists); acc = [0.0] * len(lists)
    out = []
    while True:
        best = None
        for k, l in enumerate(lists):
            if pos[k] < len(l):
                frac = (acc[k] + 0.5 * l[pos[k]][0]) / tot[k]
                if best is None or frac < best[0]:
                    best = (frac, k)
        if best is None: break
        k = best[1]
        out.append(lists[k][pos[k]][1]); acc[k] += lists[k][pos[k]][0]; pos[k] += 1
    return out

def make_kernel(T=256, RC=8, RA=16, RE=16, NP=128, NPD=128, skew=1, one_round=False, flags=None, scopes=False):
    NB = S_ // T
    CS = (DH_ ** -0.5) * math.log2(math.e)

    def kernel(x_hbm, w_hbm, wo_hbm, wr_ref, wg_hbm, wu_hbm, wd_hbm, out_hbm,
               x_s, w_s, wo_s, wg_s, wu_s, wd_s, wt_s, wp_s, wot_s, wop_s,
               xn_s, q_s, k_s, v_s, o_s, h_s, hn_s, out_s, sems):
        cps = {}
        nsem = [0]
        def start(name, src, dst):
            c = pltpu.make_async_copy(src, dst, sems.at[nsem[0]]); nsem[0] += 1
            c.start(); cps[name] = c
        start(("x", 0), x_hbm.at[pl.ds(0, T), :], x_s.at[pl.ds(0, T), :])
        for p in range(3):
            start(("w", p), w_hbm.at[:, pl.ds(p * D_, D_)], w_s.at[:, pl.ds(p * D_, D_)])
        for i in range(1, NB):
            start(("x", i), x_hbm.at[pl.ds(i * T, T), :], x_s.at[pl.ds(i * T, T), :])
            if i == 1:
                start("wo", wo_hbm, wo_s)
        start("wg", wg_hbm, wg_s); start("wu", wu_hbm, wu_s); start("wd", wd_hbm, wd_s)

        lo_mask = u32(0xFFFF); hi_mask = u32(0xFFFF0000)
        def permute_words(src_ref, base, dst_ref, dbase, j):
            for dp in range(10):
                a = src_ref[j, pl.ds(base + dp, 16, stride=20), :]
                b = src_ref[j, pl.ds(base + 10 + dp, 16, stride=20), :]
                lo = (a & lo_mask) | (b << 16)
                hi = (a >> 16) | (b & hi_mask)
                dst_ref[pl.ds(dbase + 32 * dp, 16), pl.ds(j * 128, 128)] = lo
                dst_ref[pl.ds(dbase + 32 * dp + 16, 16), pl.ds(j * 128, 128)] = hi

        def prep_w_list(p):
            L = []
            def t0():
                cps[("w", p)].wait()
            L.append((0.1, t0))
            for j in range(5):
                def t1(j=j):
                    wt = pltpu.bitcast(w_s[pl.ds(j * 128, 128), pl.ds(p * D_, D_)].T, u32)
                    wt_s[j, pl.ds(p * 320, 320), :] = wt
                L.append((1, t1))
            for j in range(5):
                L.append((1, functools.partial(permute_words, wt_s, p * 320, wp_s, p * 320, j)))
            return L

        def prep_wo_list():
            L = []
            def t0():
                cps["wo"].wait()
            L.append((0.1, t0))
            for j in range(5):
                def t1(j=j):
                    wot_s[j, :, :] = pltpu.bitcast(wo_s[:, pl.ds(j * 128, 128)], u32)
                    permute_words(wot_s, 0, wop_s, 0, j)
                L.append((1, t1))
            return L

        for j in range(5):
            k_s[j, pl.ds(0, HALO), :] = jnp.zeros((HALO, 128), f32)
            v_s[j, pl.ds(0, HALO), :] = jnp.zeros((HALO, 128), f32)

        stA = {}
        def A1(i, c):
            if c == 0: cps[("x", i)].wait()
            r0 = i * T + c * RA
            xc = x_s[pl.ds(r0, RA), :].astype(f32)
            s1 = jnp.sum(xc, axis=1, keepdims=True)
            s2 = jnp.sum(xc * xc, axis=1, keepdims=True)
            stA[(i, c)] = (s1, s2)
        def A2(i, c):
            r0 = i * T + c * RA
            s1, s2 = stA.pop((i, c))
            m = s1 * (1.0 / D_)
            var = jnp.maximum(s2 * (1.0 / D_) - m * m, 0.0)
            rs = jax.lax.rsqrt(var + EPS)
            xc = x_s[pl.ds(r0, RA), :].astype(f32)
            xn = (xc - m) * rs
            xn_s[pl.ds(r0 // 2, RA // 2), :] = pltpu.bitcast(xn.astype(bf16), u32)
        def A_list(i):
            n = T // RA; L = []
            for c in range(n + skew):
                if c < n: L.append((1, functools.partial(A1, i, c)))
                if c >= skew: L.append((1, functools.partial(A2, i, c - skew)))
            return L

        def Bp(i, n0):
            p = n0 // D_
            lhs = pltpu.bitcast(xn_s[pl.ds(i * T // 2, T // 2), :], bf16)
            rhs = pltpu.bitcast(wp_s[pl.ds(n0 // 2, NP // 2), :], bf16)
            acc = jax.lax.dot_general(lhs, rhs, NT, preferred_element_type=f32)
            for jj in range(NP // 128):
                j = ((n0 % D_) // 128) + jj
                blk = acc[:, jj * 128:(jj + 1) * 128]
                if p == 0:
                    q_s[j, pl.ds(i * T, T), :] = blk * CS
                elif p == 1:
                    k_s[j, pl.ds(HALO + i * T, T), :] = blk
                else:
                    v_s[j, pl.ds(HALO + i * T, T), :] = blk
        def B_list(i):
            return [(1, functools.partial(Bp, i, n0)) for n0 in range(0, 3 * D_, NP)]

        stC = {}
        def C1(i, c):
            r0 = i * T + c * RC
            qs = [q_s[j, pl.ds(r0, RC), :] for j in range(5)]
            res = []
            for w in range(W_):
                a = None
                for j in range(5):
                    t = qs[j] * k_s[j, pl.ds(HALO + r0 - 2 * w, RC), :]
                    a = t if a is None else a + t
                if one_round:
                    res.append((a, pltpu.roll(a, 32, 1), pltpu.roll(a, 64, 1), pltpu.roll(a, 96, 1)))
                else:
                    res.append((a, pltpu.roll(a, 64, 1)))
            stC[(1, i, c)] = res
        def C2(i, c):
            res = stC.pop((1, i, c)); out = []
            for t in res:
                if one_round:
                    out.append(((t[0] + t[1]) + (t[2] + t[3]), None))
                else:
                    a = t[0] + t[1]
                    out.append((a, pltpu.roll(a, 32, 1)))
            stC[(2, i, c)] = out
        def C3(i, c):
            r0 = i * T + c * RC
            res = stC.pop((2, i, c))
            ls = []
            for w in range(W_):
                a = res[w][0] if one_round else res[w][0] + res[w][1]
                if r0 - 2 * w < 0:
                    rows = jax.lax.broadcasted_iota(i32, (RC, 128), 0) + r0
                    a = jnp.where(rows - 2 * w >= 0, a, -1e9 * math.log2(math.e))
                ls.append(a)
            m = ls[0]
            for w in range(1, W_):
                m = jnp.maximum(m, ls[w])
            ps = [jnp.exp2(l - m) for l in ls]
            den = ps[0]
            for w in range(1, W_):
                den = den + ps[w]
            inv = 1.0 / den
            outs = []
            for j in range(5):
                a = None
                for w in range(W_):
                    t = ps[w] * v_s[j, pl.ds(HALO + r0 - 2 * w, RC), :]
                    a = t if a is None else a + t
                outs.append(a * inv)
            o = jnp.concatenate(outs, axis=1)
            if RC == 8:
                if c % 2 == 0:
                    stC[(3, i)] = o
                    return
                o = jnp.concatenate([stC.pop((3, i)), o], axis=0)
                o_s[pl.ds((r0 - 8) // 2, 8), :] = pltpu.bitcast(o.astype(bf16), u32)
            else:
                o_s[pl.ds(r0 // 2, RC // 2), :] = pltpu.bitcast(o.astype(bf16), u32)
        def C_list(i):
            n = T // RC; L = []
            for c in range(n + 2 * skew):
                if c < n: L.append((72, functools.partial(C1, i, c)))
                if skew <= c < n + skew: L.append((10, functools.partial(C2, i, c - skew)))
                if c >= 2 * skew: L.append((120, functools.partial(C3, i, c - 2 * skew)))
            return L

        def Dp(i, n0):
            lhs = pltpu.bitcast(o_s[pl.ds(i * T // 2, T // 2), :], bf16)
            rhs = pltpu.bitcast(wop_s[:, pl.ds(n0, NPD)], bf16)
            acc = jax.lax.dot_general(lhs, rhs, NN, preferred_element_type=f32)
            xr = x_s[pl.ds(i * T, T), pl.ds(n0, NPD)].astype(f32)
            h_s[pl.ds(i * T, T), pl.ds(n0, NPD)] = acc + xr
        def D_list(i):
            return [(1, functools.partial(Dp, i, n0)) for n0 in range(0, D_, NPD)]

        stE = {}; best = {}
        def E1(i, c):
            r0 = i * T + c * RE
            wr = wr_ref[...].astype(f32)
            h = h_s[pl.ds(r0, RE), :]
            s1 = jnp.sum(h, axis=1, keepdims=True)
            s2 = jnp.sum(h * h, axis=1, keepdims=True)
            s3 = jnp.sum(h * wr, axis=1, keepdims=True)
            stE[(i, c)] = (s1, s2, s3)
        def E2(i, c):
            r0 = i * T + c * RE
            s1, s2, s3 = stE.pop((i, c))
            if "swr" not in stE:
                stE["swr"] = jnp.sum(wr_ref[...].astype(f32), axis=1, keepdims=True)
            m = s1 * (1.0 / D_)
            var = jnp.maximum(s2 * (1.0 / D_) - m * m, 0.0)
            rs = jax.lax.rsqrt(var + EPS)
            r = (s3 - m * stE["swr"]) * rs
            h = h_s[pl.ds(r0, RE), :]
            hn = (h - m) * rs
            out_s[pl.ds(r0, RE), :] = (h + hn).astype(bf16)
            hn_s[pl.ds(r0, RE), :] = hn.astype(bf16)
            rb = jnp.broadcast_to(r, (RE, 128))
            for s8 in range(RE // 8):
                v = rb[s8 * 8:(s8 + 1) * 8, :]
                if "v" not in best:
                    best["v"] = v; best["i"] = jnp.full((8, 128), r0 + s8 * 8, i32)
                else:
                    upd = v > best["v"]
                    best["v"] = jnp.where(upd, v, best["v"])
                    best["i"] = jnp.where(upd, r0 + s8 * 8, best["i"])
            if c == T // RE - 1:
                cps[("o", i)] = pltpu.make_async_copy(out_s.at[pl.ds(i * T, T), :], out_hbm.at[pl.ds(i * T, T), :], sems.at[nsem[0]])
                nsem[0] += 1
                cps[("o", i)].start()
        def E_list(i):
            n = T // RE; L = []
            for c in range(n + skew):
                if c < n: L.append((1, functools.partial(E1, i, c)))
                if c >= skew: L.append((1.5, functools.partial(E2, i, c - skew)))
            return L

        cnt = [0]
        def run(L):
            for t in L:
                if scopes:
                    with jax.named_scope("s%d" % cnt[0]):
                        t()
                    cnt[0] += 1
                else:
                    t()
        run([t for _, t in A_list(0)])
        run([t for _, t in prep_w_list(0)])
        run(interleave(B_list(0)[0:5 * 128 // NP], prep_w_list(1)))
        run(interleave(B_list(0)[5 * 128 // NP:10 * 128 // NP], prep_w_list(2)))
        run(interleave(B_list(0)[10 * 128 // NP:], prep_wo_list(), A_list(1)))
        for it in range(0, NB + 1):
            M1 = D_list(it - 1) if it - 1 >= 0 else []
            M2 = B_list(it + 1) if it + 1 < NB else []
            Cl = C_list(it) if it < NB else []
            Al = A_list(it + 2) if it + 2 < NB else []
            El = E_list(it - 1) if it - 1 >= 0 else []
            nD, nBp = len(M1) * NPD, len(M2) * NP
            if M1 and M2:
                cut = int(len(Cl) * nD / (nD + nBp))
                run(interleave(M1, Cl[:cut]))
                run(interleave(M2, Cl[cut:], Al, El))
            elif M2:
                run(interleave(M2, Cl, Al))
            elif M1 and Cl:
                run(interleave(M1, Cl))
                run([t for _, t in El])
            else:
                run([t for _, t in M1]); run([t for _, t in El])
        bv = best["v"]; bi = best["i"] + jax.lax.broadcasted_iota(i32, (8, 128), 0)
        mx = jnp.max(bv, axis=0, keepdims=True)
        cand = jnp.where(bv == mx, bi, S_)
        idx = jnp.min(cand)
        base = pl.multiple_of((idx // 16) * 16, 16)
        cps["wg"].wait(); cps["wu"].wait(); cps["wd"].wait()
        xs = hn_s[pl.ds(base, 16), :]
        g = jnp.dot(xs, wg_s[...], preferred_element_type=f32)
        u = jnp.dot(xs, wu_s[...], preferred_element_type=f32)
        a = (g * jax.nn.sigmoid(g)) * u
        y = jnp.dot(a.astype(bf16), wd_s[...], preferred_element_type=f32)
        gate = jax.nn.sigmoid(mx[:, 0:1])
        rows = jax.lax.broadcasted_iota(i32, (16, D_), 0)
        og = out_s[pl.ds(base, 16), :].astype(f32)
        og = jnp.where(rows == (idx - base), og + y * gate, og)
        for i in range(NB):
            cps[("o", i)].wait()
        out_s[pl.ds(base, 16), :] = og.astype(bf16)
        c = pltpu.make_async_copy(out_s.at[pl.ds(base, 16), :], out_hbm.at[pl.ds(base, 16), :], sems.at[nsem[0]])
        c.start(); c.wait()

    def fn(A_x, A_wqkv, A_wo, B_x, B_w_r, B_w_gate, B_w_up, B_w_down):
        x = A_x.reshape(S_, D_)
        wr = B_w_r.reshape(1, D_)
        anyspec = pl.BlockSpec(memory_space=pl.ANY)
        vm = pltpu.VMEM
        out = pl.pallas_call(
            kernel,
            out_shape=jax.ShapeDtypeStruct((S_, D_), bf16),
            in_specs=[anyspec, anyspec, anyspec, pl.BlockSpec(memory_space=vm), anyspec, anyspec, anyspec],
            out_specs=anyspec,
            scratch_shapes=[
                vm((S_, D_), bf16), vm((D_, 3 * D_), bf16), vm((D_, D_), bf16),
                vm((D_, F_), bf16), vm((D_, F_), bf16), vm((F_, D_), bf16),
                vm((5, 960, 128), u32), vm((960, D_), u32), vm((5, 320, 128), u32), vm((320, D_), u32),
                vm((S_ // 2, D_), u32), vm((5, S_, 128), f32), vm((5, S_ + HALO, 128), f32), vm((5, S_ + HALO, 128), f32),
                vm((S_ // 2, D_), u32), vm((S_, D_), f32), vm((S_, D_), bf16), vm((S_, D_), bf16),
                pltpu.SemaphoreType.DMA((3 + NB + 4 + NB + 1,)),
            ],
            compiler_params=pltpu.CompilerParams(vmem_limit_bytes=110 * 2**20, flags=flags),
            name="fused",
        )(x, A_wqkv, A_wo, wr, B_w_gate, B_w_up, B_w_down)
        return out.reshape(1, S_, D_)
    return fn


_fn = make_kernel(**dict(one_round=True))


@jax.jit
def pallas_sequential_preLN__sliding_local_dilated__moe_arch_mod__prompt_kernel(
    A_x: jax.Array,
    A_wqkv: jax.Array,
    A_wo: jax.Array,
    B_x: jax.Array,
    B_w_r: jax.Array,
    B_w_gate: jax.Array,
    B_w_up: jax.Array,
    B_w_down: jax.Array,
):
    return _fn(A_x, A_wqkv, A_wo, B_x, B_w_r, B_w_gate, B_w_up, B_w_down)
```

```python
import functools, math
import jax, jax.numpy as jnp, numpy as np
from jax.experimental import pallas as pl
from jax.experimental.pallas import tpu as pltpu

S_, D_, H_, DH_, W_, F_ = 2048, 640, 32, 20, 8, 1536
HALO = 16
EPS = 1e-5
f32, bf16, u32, i32 = jnp.float32, jnp.bfloat16, jnp.uint32, jnp.int32
NT = (((1,), (1,)), ((), ()))
NN = (((1,), (0,)), ((), ()))

def interleave(*lists):
    lists = [l for l in lists if l]
    tot = [sum(w for w, _ in l) for l in lists]
    pos = [0] * len(lists); acc = [0.0] * len(lists)
    out = []
    while True:
        best = None
        for k, l in enumerate(lists):
            if pos[k] < len(l):
                frac = (acc[k] + 0.5 * l[pos[k]][0]) / tot[k]
                if best is None or frac < best[0]:
                    best = (frac, k)
        if best is None: break
        k = best[1]
        out.append(lists[k][pos[k]][1]); acc[k] += lists[k][pos[k]][0]; pos[k] += 1
    return out

def make_kernel(T=256, RC=8, RA=16, RE=16, NP=128, NPD=128, skew=1, one_round=True, flags=None,
                fastmath=True, sched=None, gate=0, gateA=0, gateE=0, gE_end=1792, gC_end=2048, MB=256, MD=256, xf=True, gfull=True, etok=0, ms=(), scopes=False, dma0=("x0", "w0", "w1", "w2", "xr", "ffn"), dmal={}):
    NB = S_ // T
    CS = (DH_ ** -0.5) * math.log2(math.e)

    def rsqrt(v):
        if not fastmath: return jax.lax.rsqrt(v)
        return jnp.exp2(-0.5 * jnp.log2(v))
    def recip(d):
        if not fastmath: return 1.0 / d
        return pltpu.reciprocal(d, approx=True)

    def kernel(x_hbm, w_hbm, wo_hbm, wr_ref, wg_hbm, wu_hbm, wd_hbm, out_hbm,
               x_s, w_s, wo_s, wg_s, wu_s, wd_s, wt_s, wp_s, wot_s, wop_s,
               hn_s, out_s, sems, *blk):
        xn_l, q_l, k_l, v_l, o_l, h_l = [blk[a * NB:(a + 1) * NB] for a in range(6)]
        cps = {}
        def start(name, src, dst, si):
            c = pltpu.make_async_copy(src, dst, sems.at[si])
            c.start(); cps.setdefault(name, []).append(c)
        done = set()
        def wait(name):
            for c in cps.pop(name): c.wait()
            done.add(name)
        XB = 256
        def dma(g):
            if g == "x0": start("x0", x_hbm.at[pl.ds(0, XB), :], x_s.at[pl.ds(0, XB), :], 0)
            elif g == "w0":
                start("w0a", w_hbm.at[pl.ds(0, 384), pl.ds(0, D_)], w_s.at[pl.ds(0, 384), pl.ds(0, D_)], 1)
                start("w0b", w_hbm.at[pl.ds(384, 256), pl.ds(0, D_)], w_s.at[pl.ds(384, 256), pl.ds(0, D_)], 2)
            elif g == "w1": start("w1", w_hbm.at[:, pl.ds(D_, D_)], w_s.at[:, pl.ds(D_, D_)], 3)
            elif g == "w2":
                start("w2", w_hbm.at[:, pl.ds(2 * D_, D_)], w_s.at[:, pl.ds(2 * D_, D_)], 4)
                start("w2", x_hbm.at[pl.ds(XB, XB), :], x_s.at[pl.ds(XB, XB), :], 4)
            elif g == "xr":
                start("xr", x_hbm.at[pl.ds(2 * XB, S_ - 2 * XB), :], x_s.at[pl.ds(2 * XB, S_ - 2 * XB), :], 5)
                start("xr", wo_hbm, wo_s, 5)
            elif g == "ffn":
                start("ffn", wg_hbm, wg_s, 6); start("ffn", wu_hbm, wu_s, 6); start("ffn", wd_hbm, wd_s, 6)
        for g in dma0: dma(g)

        om = {}
        def mstore(kind, ref, val):
            if kind not in ms:
                ref[...] = val; return
            if "m" not in om:
                z = pltpu.bitcast(x_s[pl.ds(0, 16), pl.ds(0, 128)], u32)
                om["m"] = z | u32(1)
            mm = om["m"]
            R, C_ = val.shape
            mm = jnp.concatenate([mm] * (R // 8), axis=0) if R > 8 else mm
            mm = jnp.concatenate([mm] * (C_ // 128), axis=1) if C_ > 128 else mm
            pltpu.store(ref, val, mask=mm != u32(0))
        lo_mask = u32(0xFFFF); hi_mask = u32(0xFFFF0000)
        def permute_words(src_ref, base, dst_ref, dbase, j):
            for dp in range(10):
                a = src_ref[j, pl.ds(base + dp, 16, stride=20), :]
                b = src_ref[j, pl.ds(base + 10 + dp, 16, stride=20), :]
                lo = (a & lo_mask) | (b << 16)
                hi = (a >> 16) | (b & hi_mask)
                mstore("w", dst_ref.at[pl.ds(dbase + 32 * dp, 16), pl.ds(j * 128, 128)], lo)
                mstore("w", dst_ref.at[pl.ds(dbase + 32 * dp + 16, 16), pl.ds(j * 128, 128)], hi)

        def prep_w(p, j):
            assert ("w%d" % p in done) if p > 0 else ("w0a" in done and (j < 3 or "w0b" in done))
            wt = pltpu.bitcast(w_s[pl.ds(j * 128, 128), pl.ds(p * D_, D_)].T, u32)
            wt_s[j, pl.ds(p * 320, 320), :] = wt
            permute_words(wt_s, p * 320, wp_s, p * 320, j)

        def prep_wo(j):
            assert "xr" in done
            wot_s[j, :, :] = pltpu.bitcast(wo_s[:, pl.ds(j * 128, 128)], u32)
            permute_words(wot_s, 0, wop_s, 0, j)

        for j in range(5):
            k_l[0][j, pl.ds(0, HALO), :] = jnp.zeros((HALO, 128), f32)
            v_l[0][j, pl.ds(0, HALO), :] = jnp.zeros((HALO, 128), f32)

        gm = {}; tok = {}; rel = {}
        def gated16(x, d0):
            d16 = jnp.concatenate([d0, d0], axis=0)
            m_ = (pltpu.bitcast(d16, u32) | u32(1)) != u32(0)
            return jnp.concatenate([jnp.where(m_, x[:, j * 128:(j + 1) * 128], d16) for j in range(x.shape[1] // 128)], axis=1)
        def gated1(x, dep):
            if gfull and x.shape[0] != 8: return gated16(x, dep[0:8, :128])
            top = gated(x[0:8, 0:128], dep)
            top = jnp.concatenate([top, x[0:8, 128:]], axis=1)
            return top if x.shape[0] == 8 else jnp.concatenate([top, x[8:, :]], axis=0)
        def gated(x, dep):
            key = id(dep)
            if key not in gm:
                d0 = dep[0:8, :128]
                gm[key] = (dep, (pltpu.bitcast(d0, u32) | u32(1)) != u32(0), d0)
            _, m_, d0 = gm[key]
            if x.shape[0] != 8:
                m_ = jnp.concatenate([m_] * (x.shape[0] // 8), axis=0) if False else m_
                return gated16(x, d0)
            if x.shape[1] == 128: return jnp.where(m_, x, d0)
            return jnp.concatenate([jnp.where(m_, x[:, j * 128:(j + 1) * 128], d0) for j in range(x.shape[1] // 128)], axis=1)
        stA = {}
        def A1(i, c):
            r0 = i * T + c * RA
            assert {0: "x0", 1: "w2"}.get(r0 // 256, "xr") in done
            xc = x_s[pl.ds(r0, RA), :].astype(f32)
            if ("A", i, c) in rel:
                xc = gated1(xc, tok[rel[("A", i, c)]])
            s1 = jnp.sum(xc, axis=1, keepdims=True)
            s2 = jnp.sum(xc * xc, axis=1, keepdims=True)
            stA[(i, c)] = (s1, s2, xc)
        def A2(i, c):
            r0 = i * T + c * RA
            s1, s2, xc0 = stA.pop((i, c))
            m = s1 * (1.0 / D_)
            var = jnp.maximum(s2 * (1.0 / D_) - m * m, 0.0)
            rs = rsqrt(var + EPS)
            xc = xc0 if xf else x_s[pl.ds(r0, RA), :].astype(f32)
            xn = (xc - m) * rs
            mstore("x", xn_l[i].at[pl.ds(c * RA // 2, RA // 2), :], pltpu.bitcast(xn.astype(bf16), u32))
            if gateA: stA[("g", r0 // RA)] = xn
        def A_list(i):
            n = T // RA; L = []
            if gateA:
                for c in range(n):
                    L.append((1, functools.partial(A1, i, c))); L.append((1, functools.partial(A2, i, c)))
                return L
            for c in range(n + skew):
                if c < n: L.append((1, functools.partial(A1, i, c)))
                if c >= skew: L.append((1, functools.partial(A2, i, c - skew)))
            return L

        def dst(p, j, i):
            if p == 0: return q_l[i].at[j, pl.ds(0, T), :]
            return (k_l if p == 1 else v_l)[i].at[j, pl.ds(HALO, T), :]
        def Bp(i, n0):
          p = n0 // D_
          for m0 in range(0, T, MB):
            lhs = pltpu.bitcast(xn_l[i][pl.ds(m0 // 2, MB // 2), :], bf16)
            rhs = pltpu.bitcast(wp_s[pl.ds(n0 // 2, NP // 2), :], bf16)
            acc = jax.lax.dot_general(lhs, rhs, NT, preferred_element_type=f32)
            for jj in range(NP // 128):
                j = ((n0 % D_) // 128) + jj
                blk = acc[:, jj * 128:(jj + 1) * 128]
                mstore("qkv", dst(p, j, i).at[pl.ds(m0, MB), :], blk * CS if p == 0 else blk)
                if m0 == 0: tok[("B", i, p, j)] = blk[0:8, :]
                if p > 0 and i + 1 < NB and m0 + MB == T:
                    (k_l if p == 1 else v_l)[i + 1][j, pl.ds(0, HALO), :] = blk[MB - HALO:, :]
        def B_list(i):
            return [(1, functools.partial(Bp, i, n0)) for n0 in range(0, 3 * D_, NP)]

        stC = {}
        def C1(i, c):
            r0 = i * T + c * RC
            qs = [q_l[i][j, pl.ds(c * RC, RC), :] for j in range(5)]
            if ("C", i, c) in rel:
                dep = tok[rel[("C", i, c)]]
                qs = [gated(q_, dep) if (gfull or j_ == 0) else q_ for j_, q_ in enumerate(qs)]
            for jj_, tk in enumerate(rel.get(("CE", i, c), [])):
                qs[jj_ % 5] = gated(qs[jj_ % 5], tok[tk])
            res = []
            for w in range(W_):
                a = None
                for j in range(5):
                    t = qs[j] * k_l[i][j, pl.ds(HALO + c * RC - 2 * w, RC), :]
                    a = t if a is None else a + t
                if one_round:
                    res.append((a, pltpu.roll(a, 32, 1), pltpu.roll(a, 64, 1), pltpu.roll(a, 96, 1)))
                else:
                    res.append((a, pltpu.roll(a, 64, 1)))
            stC[(1, i, c)] = res
        def C2(i, c):
            res = stC.pop((1, i, c)); out = []
            for t in res:
                if one_round:
                    out.append(((t[0] + t[1]) + (t[2] + t[3]), None))
                else:
                    a = t[0] + t[1]
                    out.append((a, pltpu.roll(a, 32, 1)))
            stC[(2, i, c)] = out
        def C3(i, c):
            r0 = i * T + c * RC
            res = stC.pop((2, i, c))
            ls = []
            for w in range(W_):
                a = res[w][0] if one_round else res[w][0] + res[w][1]
                if r0 - 2 * w < 0:
                    rows = jax.lax.broadcasted_iota(i32, (RC, 128), 0) + r0
                    a = jnp.where(rows - 2 * w >= 0, a, -1e9 * math.log2(math.e))
                ls.append(a)
            m = ls[0]
            for w in range(1, W_):
                m = jnp.maximum(m, ls[w])
            ps = [jnp.exp2(l - m) for l in ls]
            den = ps[0]
            for w in range(1, W_):
                den = den + ps[w]
            inv = recip(den)
            outs = []
            for j in range(5):
                a = None
                for w in range(W_):
                    t = ps[w] * v_l[i][j, pl.ds(HALO + c * RC - 2 * w, RC), :]
                    a = t if a is None else a + t
                outs.append(a * inv)
            if gate: stC[("g", i * (T // RC) + c)] = outs[4]
            o = jnp.concatenate(outs, axis=1)
            if RC == 8:
                if c % 2 == 0:
                    stC[(3, i)] = o
                    return
                o = jnp.concatenate([stC.pop((3, i)), o], axis=0)
                mstore("o", o_l[i].at[pl.ds((c * RC - 8) // 2, 8), :], pltpu.bitcast(o.astype(bf16), u32))
            else:
                o_l[i][pl.ds(c * RC // 2, RC // 2), :] = pltpu.bitcast(o.astype(bf16), u32)
        def C_list(i):
            n = T // RC; L = []
            if gate:
                for c in range(n):
                    L.append((72, functools.partial(C1, i, c)))
                    L.append((10, functools.partial(C2, i, c)))
                    L.append((120, functools.partial(C3, i, c)))
                return L
            for c in range(n + 2 * skew):
                if c < n: L.append((72, functools.partial(C1, i, c)))
                if skew <= c < n + skew: L.append((10, functools.partial(C2, i, c - skew)))
                if c >= 2 * skew: L.append((120, functools.partial(C3, i, c - 2 * skew)))
            return L

        def Dp(r0_, M_, n0):
          assert "Pwo" in done and all(("C", r0_ // T, c) in done for c in range(T // RC))
          M = min(M_, MD)
          for r0 in range(r0_, r0_ + M_, M):
            lhs = pltpu.bitcast(o_l[r0 // T][pl.ds((r0 % T) // 2, M // 2), :], bf16)
            rhs = pltpu.bitcast(wop_s[:, pl.ds(n0, NPD)], bf16)
            acc = jax.lax.dot_general(lhs, rhs, NN, preferred_element_type=f32)
            xr = x_s[pl.ds(r0, M), pl.ds(n0, NPD)].astype(f32)
            hh = acc + xr
            mstore("h", h_l[r0 // T].at[pl.ds(r0 % T, M), pl.ds(n0, NPD)], hh)
            tok[("D", r0, n0 // 128)] = hh[0:8, 0:128]
        def D_list(r0, M):
            return [(1, functools.partial(Dp, r0, M, n0)) for n0 in range(0, D_, NPD)]

        stE = {}; best = {}
        def E1(r0):
            if "wr" not in stE:
                stE["wr"] = jnp.broadcast_to(wr_ref[...].astype(f32).reshape(1, D_), (RE, D_))
            wr = stE["wr"]
            h = h_l[r0 // T][pl.ds(r0 % T, RE), :]
            if ("E", r0 // T, (r0 % T) // RE) in rel:
                h = gated1(h, tok[rel[("E", r0 // T, (r0 % T) // RE)]])
            s1 = jnp.sum(h, axis=1, keepdims=True)
            s2 = jnp.sum(h * h, axis=1, keepdims=True)
            s3 = jnp.sum(h * wr, axis=1, keepdims=True)
            stE[r0] = (s1, s2, s3)
        def E2(r0):
            s1, s2, s3 = stE.pop(r0)
            if "swr" not in stE:
                stE["swr"] = jnp.sum(wr_ref[...].astype(f32).reshape(1, D_), axis=1, keepdims=True)
            m = s1 * (1.0 / D_)
            var = jnp.maximum(s2 * (1.0 / D_) - m * m, 0.0)
            rs = rsqrt(var + EPS)
            r = (s3 - m * stE["swr"]) * rs
            h = h_l[r0 // T][pl.ds(r0 % T, RE), :]
            hn = (h - m) * rs
            out_s[pl.ds(r0, RE), :] = (h + hn).astype(bf16)
            hn_s[pl.ds(r0, RE), :] = hn.astype(bf16)
            rb = jnp.broadcast_to(r, (RE, 128))
            for s8 in range(RE // 8):
                v = rb[s8 * 8:(s8 + 1) * 8, :]
                if "v" not in best:
                    best["v"] = v; best["i"] = jnp.full((8, 128), r0 + s8 * 8, i32)
                else:
                    upd = v > best["v"]
                    best["v"] = jnp.where(upd, v, best["v"])
                    best["i"] = jnp.where(upd, r0 + s8 * 8, best["i"])
            tok[("E", r0 // T, (r0 % T) // RE)] = best["v"] if etok == 0 else (hn[8:16, 512:640] if etok == 1 else best["v"] + hn[8:16, 512:640])
        outcp = []
        def Eout(r0, M):
            c = pltpu.make_async_copy(out_s.at[pl.ds(r0, M), :], out_hbm.at[pl.ds(r0, M), :], sems.at[0])
            c.start(); outcp.append(c)
        def E_list(r0, M):
            n = M // RE; L = []
            if gateE and r0 < gE_end:
                for c in range(n):
                    L.append((1, functools.partial(E1, r0 + c * RE))); L.append((1, functools.partial(E2, r0 + c * RE)))
            else:
              for c in range(n + skew):
                if c < n: L.append((1, functools.partial(E1, r0 + c * RE)))
                if c >= skew: L.append((1.5, functools.partial(E2, r0 + (c - skew) * RE)))
            L.append((0.01, functools.partial(Eout, r0, M)))
            return L

        def run(L):
            for t in L: t()
        def prep_part(p):
            for j in range(5): prep_w(p, j)
        scope = [None]
        def enter(name):
            if not scopes: return
            if scope[0] is not None: scope[0].__exit__(None, None, None)
            scope[0] = jax.named_scope(name) if name else None
            if scope[0] is not None: scope[0].__enter__()
        for st in sched:
            k = st[0]
            if k == "scope": enter(st[1]); continue
            if k == "wait":
                wait(st[1])
                for g in dmal.get(st[1], ()): dma(g)
            elif k == "P":
                for j in (st[2] if len(st) > 2 else range(5)): prep_w(st[1], j)
            elif k == "Pwo":
                for j in range(5): prep_wo(j)
                done.add("Pwo")
            elif k == "A":
                run([t for _, t in A_list(st[1])])
                for c in range(T // RA): done.add(("A", st[1], c))
            elif k == "B":
                _, i, p, lo, hi = st
                assert all(("A", i, c) in done for c in range(T // RA))
                for n in range(lo, hi): done.add(("B", i, p, n))
                for n0 in range(p * D_ + lo * 128, p * D_ + hi * 128, NP): Bp(i, n0)
            elif k == "C": run([t for _, t in C_list(st[1])])
            elif k == "Cc":
                assert all(("B", st[1], p, n) in done for p in range(3) for n in range(5))
                C1(st[1], st[2]); C2(st[1], st[2]); C3(st[1], st[2]); done.add(("C", st[1], st[2]))
            elif k == "Ac": A1(st[1], st[2]); A2(st[1], st[2]); done.add(("A", st[1], st[2]))
            elif k == "Ec":
                assert all(("D", st[1], n) in done for n in range(5))
                done.add(("E", st[1], st[2]))
                E1(st[1] * T + st[2] * RE); E2(st[1] * T + st[2] * RE)
            elif k == "Eo":
                assert all(("E", st[1], c) in done for c in range(T // RE))
                Eout(st[1] * T, T)
            elif k == "Dn": Dp(st[1] * T, T, st[2] * NPD); done.add(("D", st[1], st[2]))
            elif k == "D": run([t for _, t in D_list(st[1], st[2])])
            elif k == "E": run([t for _, t in E_list(st[1], st[2])])
            elif k == "rel": rel[st[1]] = st[2]
            elif k == "rel2": rel.setdefault(st[1], []).append(st[2])
            elif k == "chain":
                for _ in range(st[1]):
                    best["v"] = pltpu.roll(best["v"], 64, 1)
            else: raise ValueError(k)
        enter("tail")
        bv = best["v"]; bi = best["i"] + jax.lax.broadcasted_iota(i32, (8, 128), 0)
        mx = jnp.max(bv, axis=0, keepdims=True)
        cand = jnp.where(bv == mx, bi, S_)
        idx = jnp.min(cand)
        base = pl.multiple_of((idx // 16) * 16, 16)
        wait("ffn")
        xs = hn_s[pl.ds(base, 16), :]
        g = jnp.dot(xs, wg_s[...], preferred_element_type=f32)
        u = jnp.dot(xs, wu_s[...], preferred_element_type=f32)
        a = (g * jax.nn.sigmoid(g)) * u
        y = jnp.dot(a.astype(bf16), wd_s[...], preferred_element_type=f32)
        gsig = jax.nn.sigmoid(mx[:, 0:1])
        rows = jax.lax.broadcasted_iota(i32, (16, D_), 0)
        og = out_s[pl.ds(base, 16), :].astype(f32)
        og = jnp.where(rows == (idx - base), og + y * gsig, og)
        for c in outcp: c.wait()
        out_s[pl.ds(base, 16), :] = og.astype(bf16)
        c = pltpu.make_async_copy(out_s.at[pl.ds(base, 16), :], out_hbm.at[pl.ds(base, 16), :], sems.at[1])
        c.start(); c.wait()
        enter(None)

    def fn(A_x, A_wqkv, A_wo, B_x, B_w_r, B_w_gate, B_w_up, B_w_down):
        x = A_x.reshape(S_, D_)
        anyspec = pl.BlockSpec(memory_space=pl.ANY)
        vm = pltpu.VMEM
        out = pl.pallas_call(
            kernel,
            out_shape=jax.ShapeDtypeStruct((S_, D_), bf16),
            in_specs=[anyspec, anyspec, anyspec, pl.BlockSpec(memory_space=vm), anyspec, anyspec, anyspec],
            out_specs=anyspec,
            scratch_shapes=[
                vm((S_, D_), bf16), vm((D_, 3 * D_), bf16), vm((D_, D_), bf16),
                vm((D_, F_), bf16), vm((D_, F_), bf16), vm((F_, D_), bf16),
                vm((5, 960, 128), u32), vm((960, D_), u32), vm((5, 320, 128), u32), vm((320, D_), u32),
                vm((S_, D_), bf16), vm((S_, D_), bf16),
                pltpu.SemaphoreType.DMA((7,)),
            ] + [vm((T // 2, D_), u32) for _ in range(NB)] + [vm((5, T, 128), f32) for _ in range(NB)]
              + [vm((5, T + HALO, 128), f32) for _ in range(2 * NB)]
              + [vm((T // 2, D_), u32) for _ in range(NB)] + [vm((T, D_), f32) for _ in range(NB)],
            compiler_params=pltpu.CompilerParams(vmem_limit_bytes=110 * 2**20, flags=flags),
            name="fused",
        )(x, A_wqkv, A_wo, B_w_r, B_w_gate, B_w_up, B_w_down)
        return out.reshape(1, S_, D_)
    return fn


def mk_sched(DD=3, T=128, split=3, wpos=11, pwo=4, cspan=20, espan=20, aspan=14, coff=0, eoff=0, aoff=0, RC=8, elag=3, dgrp=1, endsh=0):
    NB = S_ // T
    u0 = 256 // T
    nC, nE, nA = T // RC, T // 16, T // 16
    L = [("scope", "s0_x0"), ("wait", "x0")] + [("A", i) for i in range(u0)]
    L += [("scope", "s1_w0"), ("wait", "w0a"), ("P", 0, (0, 1, 2)), ("wait", "w0b"), ("P", 0, (3, 4))]
    def Bs(p, lo, hi): return [("B", i, p, n, n + 1) for n in range(lo, hi) for i in range(u0)]
    L += [("scope", "s2_q")] + Bs(0, 0, split) + [("scope", "s3_wk"), ("wait", "w1"), ("P", 1)] + Bs(0, split, 5)
    L += Bs(1, 0, split) + [("scope", "s4_wv"), ("wait", "w2"), ("P", 2)] + [("A", i) for i in range(u0, 2 * u0)] + Bs(1, split, 5)
    L += Bs(2, 0, 5)
    slots = []
    seq = [(p, n) for p in range(3) for n in range(5)]
    for i in range(u0, NB):
        for (p, n) in seq: slots.append(("B", i, p, n))
        if i >= NB - 1 - endsh and endsh > 0: continue
        if i - DD >= 0 and (i - DD) % dgrp == dgrp - 1:
            for d in range(i - DD - dgrp + 1, i - DD + 1):
                for n in range(5): slots.append(("D", d, n))
    nd = len([1 for sl in slots if sl[0] == "D"]) // 5
    for d in range(nd, NB):
        for n in range(5): slots.append(("D", d, n))
    pos = {sl: k for k, sl in enumerate(slots)}
    tasks = {k: [] for k in range(-1, len(slots))}
    def key(sl): return ("B", sl[1], sl[2], sl[3]) if sl[0] == "B" else ("D", sl[1] * T, sl[2])
    def add(k, kind, u, c):
        k = min(k, len(slots) - 1)
        if k >= 0: tasks[k].append(("rel", (kind, u, c), key(slots[k])))
        tasks[k].append((kind + "c", u, c))
    for u in range(NB):
        s0 = pos[("B", u, 2, 4)] if u >= u0 else -1
        dl = pos[("D", u, 0)] - 2
        if u < u0: s0 = max(0, u * cspan // 2)
        elif u < 2 * u0: s0 = max(s0, (u) * cspan // 2)
        span = min(cspan, dl - s0)
        for c in range(nC): add(s0 + coff + (c * span) // nC, "C", u, c)
    for d in range(NB):
        s0 = pos[("D", d, 4)]
        last = d == NB - 1
        span = min(espan, len(slots) - 1 - s0)
        for c in range(nE):
            add(s0 + (eoff if span > eoff else 0) + (c * max(span - eoff, 0)) // nE, "E", d, c)
        k = s0 + (eoff if span > eoff else 0) + ((nE - 1) * max(span - eoff, 0)) // nE
        tasks[min(k, len(slots) - 1)].append(("Eo", d))
    for a_ in range(2 * u0, NB):
        s1 = pos[("B", a_, 0, 0)]
        s0 = s1 - 20 + aoff if a_ >= 3 * u0 else (pos[("B", 2 * u0 - 1) + seq[wpos]] if wpos < 15 else pos[("D", 0, wpos - 15)])
        span = aspan if a_ >= 3 * u0 else max(1, (s1 - 3 - s0) if a_ == 2 * u0 else 10)
        for c in range(nA): add(s0 + (c * span) // nA, "A", a_, c)
    if elag is not None:
        for k in range(len(slots)):
            for t in list(tasks[k]):
                if t[0] == "Ec":
                    done = False
                    for k2 in range(k + elag, len(slots)):
                        for t2 in tasks[k2]:
                            if t2[0] == "Cc":
                                pos2 = tasks[k2].index(t2)
                                tasks[k2].insert(pos2, ("rel2", ("CE", t2[1], t2[2]), ("E", t[1], t[2])))
                                done = True; break
                        if done: break
    L += tasks[-1]
    for k, sl in enumerate(slots):
        if sl[0] == "B" and sl[2:] == (0, 0): L.append(("scope", "u%02d" % sl[1]))
        if sl[0] == "D" and sl[1] == NB - DD and sl[2] == 0: L.append(("scope", "v_endD"))
        if sl[0] == "B":
            if sl[1] == 2 * u0 - 1 and seq.index(sl[2:]) == wpos: L += [("wait", "xr"), ("Pwo",)]
            L.append(("B", sl[1], sl[2], sl[3], sl[3] + 1))
        else:
            if wpos >= 15 and sl[1] == 0 and sl[2] == wpos - 15: L.append(("wait", "xr"))
            L.append(("Dn", sl[1], sl[2]))
        L += tasks[k]
    return L

def mk(DD=3, split=3, wpos=11, pwo=4, cspan=20, espan=20, aspan=14, coff=0, eoff=0, aoff=0, elag=3, dgrp=1, endsh=0, **kw):
    kw.setdefault("T", 128); kw.setdefault("MB", 128); kw.setdefault("MD", 128)
    T = kw["T"]
    return make_kernel(sched=mk_sched(DD, T, split, wpos, pwo, cspan, espan, aspan, coff, eoff, aoff, kw.get("RC", 8), elag, dgrp, endsh), **kw)


_fn = mk(**dict(elag=None,ms=('x','h','o'),endsh=2))


@jax.jit
def pallas_sequential_preLN__sliding_local_dilated__moe_arch_mod__prompt_kernel(
    A_x: jax.Array,
    A_wqkv: jax.Array,
    A_wo: jax.Array,
    B_x: jax.Array,
    B_w_r: jax.Array,
    B_w_gate: jax.Array,
    B_w_up: jax.Array,
    B_w_down: jax.Array,
):
    return _fn(A_x, A_wqkv, A_wo, B_x, B_w_r, B_w_gate, B_w_up, B_w_down)
```

```python
import functools, math
import jax, jax.numpy as jnp, numpy as np
from jax.experimental import pallas as pl
from jax.experimental.pallas import tpu as pltpu

S_, D_, H_, DH_, W_, F_ = 2048, 640, 32, 20, 8, 1536
HALO = 16
EPS = 1e-5
f32, bf16, u32, i32 = jnp.float32, jnp.bfloat16, jnp.uint32, jnp.int32
NT = (((1,), (1,)), ((), ()))
NN = (((1,), (0,)), ((), ()))

def interleave(*lists):
    lists = [l for l in lists if l]
    tot = [sum(w for w, _ in l) for l in lists]
    pos = [0] * len(lists); acc = [0.0] * len(lists)
    out = []
    while True:
        best = None
        for k, l in enumerate(lists):
            if pos[k] < len(l):
                frac = (acc[k] + 0.5 * l[pos[k]][0]) / tot[k]
                if best is None or frac < best[0]:
                    best = (frac, k)
        if best is None: break
        k = best[1]
        out.append(lists[k][pos[k]][1]); acc[k] += lists[k][pos[k]][0]; pos[k] += 1
    return out

def make_kernel(T=256, RC=8, RA=16, RE=16, NP=128, NPD=128, skew=1, one_round=True, flags=None,
                fastmath=True, sched=None, gate=0, gateA=0, gateE=0, gE_end=1792, gC_end=2048, MB=256, MD=256, xf=True):
    NB = S_ // T
    CS = (DH_ ** -0.5) * math.log2(math.e)

    def rsqrt(v):
        if not fastmath: return jax.lax.rsqrt(v)
        return jnp.exp2(-0.5 * jnp.log2(v))
    def recip(d):
        if not fastmath: return 1.0 / d
        return pltpu.reciprocal(d, approx=True)

    def kernel(x_hbm, w_hbm, wo_hbm, wr_ref, wg_hbm, wu_hbm, wd_hbm, out_hbm,
               x_s, w_s, wo_s, wg_s, wu_s, wd_s, wt_s, wp_s, wot_s, wop_s,
               hn_s, out_s, sems, *blk):
        xn_l, q_l, k_l, v_l, o_l, h_l = [blk[a * NB:(a + 1) * NB] for a in range(6)]
        cps = {}
        def start(name, src, dst, si):
            c = pltpu.make_async_copy(src, dst, sems.at[si])
            c.start(); cps.setdefault(name, []).append(c)
        def wait(name):
            for c in cps.pop(name): c.wait()
        XB = 256
        start("x0", x_hbm.at[pl.ds(0, XB), :], x_s.at[pl.ds(0, XB), :], 0)
        start("w0a", w_hbm.at[pl.ds(0, 384), pl.ds(0, D_)], w_s.at[pl.ds(0, 384), pl.ds(0, D_)], 1)
        start("w0b", w_hbm.at[pl.ds(384, 256), pl.ds(0, D_)], w_s.at[pl.ds(384, 256), pl.ds(0, D_)], 2)
        start("w1", w_hbm.at[:, pl.ds(D_, D_)], w_s.at[:, pl.ds(D_, D_)], 3)
        start("w2", w_hbm.at[:, pl.ds(2 * D_, D_)], w_s.at[:, pl.ds(2 * D_, D_)], 4)
        start("w2", x_hbm.at[pl.ds(XB, XB), :], x_s.at[pl.ds(XB, XB), :], 4)
        start("xr", x_hbm.at[pl.ds(2 * XB, S_ - 2 * XB), :], x_s.at[pl.ds(2 * XB, S_ - 2 * XB), :], 5)
        start("xr", wo_hbm, wo_s, 5)
        start("ffn", wg_hbm, wg_s, 6); start("ffn", wu_hbm, wu_s, 6); start("ffn", wd_hbm, wd_s, 6)

        lo_mask = u32(0xFFFF); hi_mask = u32(0xFFFF0000)
        def permute_words(src_ref, base, dst_ref, dbase, j):
            for dp in range(10):
                a = src_ref[j, pl.ds(base + dp, 16, stride=20), :]
                b = src_ref[j, pl.ds(base + 10 + dp, 16, stride=20), :]
                lo = (a & lo_mask) | (b << 16)
                hi = (a >> 16) | (b & hi_mask)
                dst_ref[pl.ds(dbase + 32 * dp, 16), pl.ds(j * 128, 128)] = lo
                dst_ref[pl.ds(dbase + 32 * dp + 16, 16), pl.ds(j * 128, 128)] = hi

        def prep_w(p, j):
            assert ("w%d" % p not in cps) and (p > 0 or ("w0a" not in cps and (j < 3 or "w0b" not in cps)))
            wt = pltpu.bitcast(w_s[pl.ds(j * 128, 128), pl.ds(p * D_, D_)].T, u32)
            wt_s[j, pl.ds(p * 320, 320), :] = wt
            permute_words(wt_s, p * 320, wp_s, p * 320, j)

        def prep_wo(j):
            assert "xr" not in cps
            wot_s[j, :, :] = pltpu.bitcast(wo_s[:, pl.ds(j * 128, 128)], u32)
            permute_words(wot_s, 0, wop_s, 0, j)

        for j in range(5):
            k_l[0][j, pl.ds(0, HALO), :] = jnp.zeros((HALO, 128), f32)
            v_l[0][j, pl.ds(0, HALO), :] = jnp.zeros((HALO, 128), f32)

        gm = {}; tok = {}; rel = {}
        def gated16(x, d0):
            d16 = jnp.concatenate([d0, d0], axis=0)
            m_ = (pltpu.bitcast(d16, u32) | u32(1)) != u32(0)
            return jnp.concatenate([jnp.where(m_, x[:, j * 128:(j + 1) * 128], d16) for j in range(x.shape[1] // 128)], axis=1)
        def gated(x, dep):
            key = id(dep)
            if key not in gm:
                d0 = dep[0:8, :128]
                gm[key] = (dep, (pltpu.bitcast(d0, u32) | u32(1)) != u32(0), d0)
            _, m_, d0 = gm[key]
            if x.shape[0] != 8:
                m_ = jnp.concatenate([m_] * (x.shape[0] // 8), axis=0) if False else m_
                return gated16(x, d0)
            if x.shape[1] == 128: return jnp.where(m_, x, d0)
            return jnp.concatenate([jnp.where(m_, x[:, j * 128:(j + 1) * 128], d0) for j in range(x.shape[1] // 128)], axis=1)
        stA = {}
        def A1(i, c):
            r0 = i * T + c * RA
            assert {0: "x0", 1: "w2"}.get(r0 // 256, "xr") not in cps
            xc = x_s[pl.ds(r0, RA), :].astype(f32)
            if gateA:
                dep = None
                if c >= gateA: dep = stA.pop(("g", r0 // RA - gateA))
                elif ("A", i) in rel: dep = tok[rel[("A", i)]]
                if dep is not None: xc = gated(xc, dep)
            s1 = jnp.sum(xc, axis=1, keepdims=True)
            s2 = jnp.sum(xc * xc, axis=1, keepdims=True)
            stA[(i, c)] = (s1, s2, xc)
        def A2(i, c):
            r0 = i * T + c * RA
            s1, s2, xc0 = stA.pop((i, c))
            m = s1 * (1.0 / D_)
            var = jnp.maximum(s2 * (1.0 / D_) - m * m, 0.0)
            rs = rsqrt(var + EPS)
            xc = xc0 if xf else x_s[pl.ds(r0, RA), :].astype(f32)
            xn = (xc - m) * rs
            xn_l[i][pl.ds(c * RA // 2, RA // 2), :] = pltpu.bitcast(xn.astype(bf16), u32)
            if gateA: stA[("g", r0 // RA)] = xn
        def A_list(i):
            n = T // RA; L = []
            if gateA:
                for c in range(n):
                    L.append((1, functools.partial(A1, i, c))); L.append((1, functools.partial(A2, i, c)))
                return L
            for c in range(n + skew):
                if c < n: L.append((1, functools.partial(A1, i, c)))
                if c >= skew: L.append((1, functools.partial(A2, i, c - skew)))
            return L

        def dst(p, j, i):
            if p == 0: return q_l[i].at[j, pl.ds(0, T), :]
            return (k_l if p == 1 else v_l)[i].at[j, pl.ds(HALO, T), :]
        def Bp(i, n0):
          p = n0 // D_
          for m0 in range(0, T, MB):
            lhs = pltpu.bitcast(xn_l[i][pl.ds(m0 // 2, MB // 2), :], bf16)
            rhs = pltpu.bitcast(wp_s[pl.ds(n0 // 2, NP // 2), :], bf16)
            acc = jax.lax.dot_general(lhs, rhs, NT, preferred_element_type=f32)
            for jj in range(NP // 128):
                j = ((n0 % D_) // 128) + jj
                blk = acc[:, jj * 128:(jj + 1) * 128]
                dst(p, j, i)[pl.ds(m0, MB), :] = blk * CS if p == 0 else blk
                if m0 == 0: tok[("B", i, p, j)] = blk[0:8, :]
                if p > 0 and i + 1 < NB and m0 + MB == T:
                    (k_l if p == 1 else v_l)[i + 1][j, pl.ds(0, HALO), :] = blk[MB - HALO:, :]
        def B_list(i):
            return [(1, functools.partial(Bp, i, n0)) for n0 in range(0, 3 * D_, NP)]

        stC = {}
        def C1(i, c):
            r0 = i * T + c * RC
            qs = [q_l[i][j, pl.ds(c * RC, RC), :] for j in range(5)]
            if gate and r0 < gC_end:
                dep = None
                if c >= gate: dep = stC.pop(("g", i * (T // RC) + c - gate))
                elif ("C", i) in rel: dep = tok[rel[("C", i)]]
                if dep is not None: qs = [gated(q_, dep) for q_ in qs]
            res = []
            for w in range(W_):
                a = None
                for j in range(5):
                    t = qs[j] * k_l[i][j, pl.ds(HALO + c * RC - 2 * w, RC), :]
                    a = t if a is None else a + t
                if one_round:
                    res.append((a, pltpu.roll(a, 32, 1), pltpu.roll(a, 64, 1), pltpu.roll(a, 96, 1)))
                else:
                    res.append((a, pltpu.roll(a, 64, 1)))
            stC[(1, i, c)] = res
        def C2(i, c):
            res = stC.pop((1, i, c)); out = []
            for t in res:
                if one_round:
                    out.append(((t[0] + t[1]) + (t[2] + t[3]), None))
                else:
                    a = t[0] + t[1]
                    out.append((a, pltpu.roll(a, 32, 1)))
            stC[(2, i, c)] = out
        def C3(i, c):
            r0 = i * T + c * RC
            res = stC.pop((2, i, c))
            ls = []
            for w in range(W_):
                a = res[w][0] if one_round else res[w][0] + res[w][1]
                if r0 - 2 * w < 0:
                    rows = jax.lax.broadcasted_iota(i32, (RC, 128), 0) + r0
                    a = jnp.where(rows - 2 * w >= 0, a, -1e9 * math.log2(math.e))
                ls.append(a)
            m = ls[0]
            for w in range(1, W_):
                m = jnp.maximum(m, ls[w])
            ps = [jnp.exp2(l - m) for l in ls]
            den = ps[0]
            for w in range(1, W_):
                den = den + ps[w]
            inv = recip(den)
            outs = []
            for j in range(5):
                a = None
                for w in range(W_):
                    t = ps[w] * v_l[i][j, pl.ds(HALO + c * RC - 2 * w, RC), :]
                    a = t if a is None else a + t
                outs.append(a * inv)
            if gate: stC[("g", i * (T // RC) + c)] = outs[4]
            o = jnp.concatenate(outs, axis=1)
            if RC == 8:
                if c % 2 == 0:
                    stC[(3, i)] = o
                    return
                o = jnp.concatenate([stC.pop((3, i)), o], axis=0)
                o_l[i][pl.ds((c * RC - 8) // 2, 8), :] = pltpu.bitcast(o.astype(bf16), u32)
            else:
                o_l[i][pl.ds(c * RC // 2, RC // 2), :] = pltpu.bitcast(o.astype(bf16), u32)
        def C_list(i):
            n = T // RC; L = []
            if gate:
                for c in range(n):
                    L.append((72, functools.partial(C1, i, c)))
                    L.append((10, functools.partial(C2, i, c)))
                    L.append((120, functools.partial(C3, i, c)))
                return L
            for c in range(n + 2 * skew):
                if c < n: L.append((72, functools.partial(C1, i, c)))
                if skew <= c < n + skew: L.append((10, functools.partial(C2, i, c - skew)))
                if c >= 2 * skew: L.append((120, functools.partial(C3, i, c - 2 * skew)))
            return L

        def Dp(r0_, M_, n0):
          M = min(M_, MD)
          for r0 in range(r0_, r0_ + M_, M):
            lhs = pltpu.bitcast(o_l[r0 // T][pl.ds((r0 % T) // 2, M // 2), :], bf16)
            rhs = pltpu.bitcast(wop_s[:, pl.ds(n0, NPD)], bf16)
            acc = jax.lax.dot_general(lhs, rhs, NN, preferred_element_type=f32)
            xr = x_s[pl.ds(r0, M), pl.ds(n0, NPD)].astype(f32)
            hh = acc + xr
            h_l[r0 // T][pl.ds(r0 % T, M), pl.ds(n0, NPD)] = hh
            tok[("D", r0, n0 // 128)] = hh[0:8, 0:128]
        def D_list(r0, M):
            return [(1, functools.partial(Dp, r0, M, n0)) for n0 in range(0, D_, NPD)]

        stE = {}; best = {}
        def E1(r0):
            if "wr" not in stE:
                stE["wr"] = jnp.broadcast_to(wr_ref[...].astype(f32).reshape(1, D_), (RE, D_))
            wr = stE["wr"]
            h = h_l[r0 // T][pl.ds(r0 % T, RE), :]
            if gateE and r0 < gE_end:
                dep = None
                c = (r0 % T) // RE
                if c >= gateE: dep = stE.pop(("g", r0 // RE - gateE))
                elif ("E", r0 // T) in rel: dep = tok[rel[("E", r0 // T)]]
                if dep is not None: h = gated(h, dep)
            s1 = jnp.sum(h, axis=1, keepdims=True)
            s2 = jnp.sum(h * h, axis=1, keepdims=True)
            s3 = jnp.sum(h * wr, axis=1, keepdims=True)
            stE[r0] = (s1, s2, s3)
        def E2(r0):
            s1, s2, s3 = stE.pop(r0)
            if "swr" not in stE:
                stE["swr"] = jnp.sum(wr_ref[...].astype(f32).reshape(1, D_), axis=1, keepdims=True)
            m = s1 * (1.0 / D_)
            var = jnp.maximum(s2 * (1.0 / D_) - m * m, 0.0)
            rs = rsqrt(var + EPS)
            r = (s3 - m * stE["swr"]) * rs
            h = h_l[r0 // T][pl.ds(r0 % T, RE), :]
            hn = (h - m) * rs
            out_s[pl.ds(r0, RE), :] = (h + hn).astype(bf16)
            hn_s[pl.ds(r0, RE), :] = hn.astype(bf16)
            if gateE: stE[("g", r0 // RE)] = hn
            rb = jnp.broadcast_to(r, (RE, 128))
            for s8 in range(RE // 8):
                v = rb[s8 * 8:(s8 + 1) * 8, :]
                if "v" not in best:
                    best["v"] = v; best["i"] = jnp.full((8, 128), r0 + s8 * 8, i32)
                else:
                    upd = v > best["v"]
                    best["v"] = jnp.where(upd, v, best["v"])
                    best["i"] = jnp.where(upd, r0 + s8 * 8, best["i"])
        outcp = []
        def Eout(r0, M):
            c = pltpu.make_async_copy(out_s.at[pl.ds(r0, M), :], out_hbm.at[pl.ds(r0, M), :], sems.at[0])
            c.start(); outcp.append(c)
        def E_list(r0, M):
            n = M // RE; L = []
            if gateE and r0 < gE_end:
                for c in range(n):
                    L.append((1, functools.partial(E1, r0 + c * RE))); L.append((1, functools.partial(E2, r0 + c * RE)))
            else:
              for c in range(n + skew):
                if c < n: L.append((1, functools.partial(E1, r0 + c * RE)))
                if c >= skew: L.append((1.5, functools.partial(E2, r0 + (c - skew) * RE)))
            L.append((0.01, functools.partial(Eout, r0, M)))
            return L

        def run(L):
            for t in L: t()
        def prep_part(p):
            for j in range(5): prep_w(p, j)
        for st in sched:
            k = st[0]
            if k == "wait": wait(st[1])
            elif k == "P":
                for j in (st[2] if len(st) > 2 else range(5)): prep_w(st[1], j)
            elif k == "Pwo":
                for j in range(5): prep_wo(j)
            elif k == "A": run([t for _, t in A_list(st[1])])
            elif k == "B":
                _, i, p, lo, hi = st
                for n0 in range(p * D_ + lo * 128, p * D_ + hi * 128, NP): Bp(i, n0)
            elif k == "C": run([t for _, t in C_list(st[1])])
            elif k == "D": run([t for _, t in D_list(st[1], st[2])])
            elif k == "E": run([t for _, t in E_list(st[1], st[2])])
            elif k == "rel": rel[(st[1], st[2])] = st[3]
            elif k == "chain":
                for _ in range(st[1]):
                    best["v"] = pltpu.roll(best["v"], 64, 1)
            else: raise ValueError(k)
        bv = best["v"]; bi = best["i"] + jax.lax.broadcasted_iota(i32, (8, 128), 0)
        mx = jnp.max(bv, axis=0, keepdims=True)
        cand = jnp.where(bv == mx, bi, S_)
        idx = jnp.min(cand)
        base = pl.multiple_of((idx // 16) * 16, 16)
        wait("ffn")
        xs = hn_s[pl.ds(base, 16), :]
        g = jnp.dot(xs, wg_s[...], preferred_element_type=f32)
        u = jnp.dot(xs, wu_s[...], preferred_element_type=f32)
        a = (g * jax.nn.sigmoid(g)) * u
        y = jnp.dot(a.astype(bf16), wd_s[...], preferred_element_type=f32)
        gsig = jax.nn.sigmoid(mx[:, 0:1])
        rows = jax.lax.broadcasted_iota(i32, (16, D_), 0)
        og = out_s[pl.ds(base, 16), :].astype(f32)
        og = jnp.where(rows == (idx - base), og + y * gsig, og)
        for c in outcp: c.wait()
        out_s[pl.ds(base, 16), :] = og.astype(bf16)
        c = pltpu.make_async_copy(out_s.at[pl.ds(base, 16), :], out_hbm.at[pl.ds(base, 16), :], sems.at[1])
        c.start(); c.wait()

    def fn(A_x, A_wqkv, A_wo, B_x, B_w_r, B_w_gate, B_w_up, B_w_down):
        x = A_x.reshape(S_, D_)
        anyspec = pl.BlockSpec(memory_space=pl.ANY)
        vm = pltpu.VMEM
        out = pl.pallas_call(
            kernel,
            out_shape=jax.ShapeDtypeStruct((S_, D_), bf16),
            in_specs=[anyspec, anyspec, anyspec, pl.BlockSpec(memory_space=vm), anyspec, anyspec, anyspec],
            out_specs=anyspec,
            scratch_shapes=[
                vm((S_, D_), bf16), vm((D_, 3 * D_), bf16), vm((D_, D_), bf16),
                vm((D_, F_), bf16), vm((D_, F_), bf16), vm((F_, D_), bf16),
                vm((5, 960, 128), u32), vm((960, D_), u32), vm((5, 320, 128), u32), vm((320, D_), u32),
                vm((S_, D_), bf16), vm((S_, D_), bf16),
                pltpu.SemaphoreType.DMA((7,)),
            ] + [vm((T // 2, D_), u32) for _ in range(NB)] + [vm((5, T, 128), f32) for _ in range(NB)]
              + [vm((5, T + HALO, 128), f32) for _ in range(2 * NB)]
              + [vm((T // 2, D_), u32) for _ in range(NB)] + [vm((T, D_), f32) for _ in range(NB)],
            compiler_params=pltpu.CompilerParams(vmem_limit_bytes=110 * 2**20, flags=flags),
            name="fused",
        )(x, A_wqkv, A_wo, B_w_r, B_w_gate, B_w_up, B_w_down)
        return out.reshape(1, S_, D_)
    return fn


def mk_sched(DD=2, lastsplit=2, T=256, split=3, rC=0, rE=0, rA=0, wpos=11, pwo=3):
    NB = S_ // T
    u0 = 256 // T
    L = [("wait", "x0")] + [("A", i) for i in range(u0)]
    L += [("wait", "w0a"), ("P", 0, (0, 1, 2)), ("wait", "w0b"), ("P", 0, (3, 4))]
    def Bs(p, lo, hi): return [("B", i, p, n, n + 1) for n in range(lo, hi) for i in range(u0)]
    L += Bs(0, 0, split) + [("wait", "w1"), ("P", 1)] + Bs(0, split, 5)
    L += Bs(1, 0, split) + [("wait", "w2"), ("P", 2)] + [("A", i) for i in range(u0, 2 * u0)] + Bs(1, split, 5)
    L += Bs(2, 0, 5)
    nd = 0
    seq = [(p, n) for p in range(3) for n in range(5)]
    cnext = 0
    for i in range(u0, NB):
        pend = []
        def rel(r, steps):
            pend.append((r if r is not None else -1, r, steps))
        cl = []
        while cnext <= i - 1 and len(cl) < (2 if i - 1 - cnext >= 1 else 1):
            cl.append(("C", cnext)); cnext += 1
        rel(rC, cl)
        d = i - 1 - DD
        if d >= 0: rel(rE, [("E", d * T, T)])
        if i + 1 < NB and i + 1 >= 3 * u0: rel(rA, [("A", i + 1)])
        for k in range(-1, 15):
            if k >= 0:
                p, n = seq[k]
                if i == 2 * u0 - 1 and k == wpos:
                    L += [("wait", "xr")] + [("A", a) for a in range(2 * u0, 3 * u0)]
                if i == pwo and k == 1: L += [("Pwo",)]
                L.append(("B", i, p, n, n + 1))
            for (kk, r, steps) in pend:
                if kk == k:
                    for st in steps:
                        if r is not None:
                            L.append(("rel", st[0], st[1] // T if st[0] == "E" else st[1], ("B", i) + seq[r]))
                        L.append(st)
        d = i - DD
        if d >= 0:
            L.append(("D", d * T, T)); nd = d + 1
    while cnext < NB:
        L.append(("C", cnext)); cnext += 1
    pendE = [d for d in range(max(0, NB - 1 - DD), nd)]
    for d in range(nd, NB):
        if d == NB - 1 and lastsplit > 1:
            m = T // lastsplit
            for s_ in range(lastsplit):
                L += [("D", d * T + s_ * m, m)]
                if s_ == 0:
                    while pendE: L.append(("E", pendE.pop(0) * T, T))
                L += [("E", d * T + s_ * m, m)]
        else:
            L += [("D", d * T, T)]
            if pendE: L.append(("E", pendE.pop(0) * T, T))
            pendE.append(d)
    while pendE: L.append(("E", pendE.pop(0) * T, T))
    return L

def mk(DD=2, lastsplit=2, split=3, rC=0, rE=0, rA=0, wpos=11, pwo=None, **kw):
    T = kw.get("T", 256)
    kw.setdefault("gE_end", S_ - T)
    if pwo is None: pwo = 2 * 256 // T
    return make_kernel(sched=mk_sched(DD, lastsplit, T, split, rC, rE, rA, wpos, pwo), **kw)


_fn = mk(**dict(MB=128,MD=128,T=128,DD=5,gate=3,gateE=2,rA=None,lastsplit=1))


@jax.jit
def pallas_sequential_preLN__sliding_local_dilated__moe_arch_mod__prompt_kernel(
    A_x: jax.Array,
    A_wqkv: jax.Array,
    A_wo: jax.Array,
    B_x: jax.Array,
    B_w_r: jax.Array,
    B_w_gate: jax.Array,
    B_w_up: jax.Array,
    B_w_down: jax.Array,
):
    return _fn(A_x, A_wqkv, A_wo, B_x, B_w_r, B_w_gate, B_w_up, B_w_down)
```
